```python
import os as _os
_os.environ.setdefault('JAX_PLATFORMS', 'cpu')
import jax
import jax.numpy as jnp

def _softmax(x, axis=-1):
    return jax.nn.softmax(x, axis=axis)

def _gelu(x):
    return jax.nn.gelu(x, approximate=True)

def _silu(x):
    return jax.nn.silu(x)

def _sigmoid(x):
    return jax.nn.sigmoid(x)

def _layernorm(x, axis=-1, eps=1e-05):
    m = jnp.mean(x, axis=axis, keepdims=True)
    v = jnp.var(x, axis=axis, keepdims=True)
    return (x - m) / jnp.sqrt(v + eps)

def _scatter_add(tgt, idx, src, axis=0):
    return tgt.at[idx].add(src)

def _segment_sum(src, seg, n):
    return jax.ops.segment_sum(src, seg, n)

class _Rng:

    def __init__(self, key):
        self._k = key

    def _next(self):
        self._k, sub = jax.random.split(self._k)
        return sub

    def normal(self, shape):
        return jax.random.normal(self._next(), shape, dtype=jnp.bfloat16)

    def randint(self, lo, hi, shape):
        return jax.random.randint(self._next(), shape, lo, hi, dtype=jnp.int32)

    def uniform(self, shape, lo=0.0, hi=1.0):
        return jax.random.uniform(self._next(), shape, jnp.bfloat16, lo, hi)

    def permutation(self, n):
        return jax.random.permutation(self._next(), n)
kernel_name = 'adaLN_cond__grouped_kv_mqa__swiglu_ffn__prompt'

def setup_inputs():
    _rng = _Rng(jax.random.key(int.from_bytes(__import__("os").urandom(4), "little")))
    _w = lambda a: (lambda t: t.astype(jnp.bfloat16) if jnp.issubdtype(t.dtype, jnp.floating) else t)(jnp.asarray(a))

    def _A_setup():
        B, S, D, H = (1, 2048, 576, 32)
        Dh = D // H
        return {'x': _w((lambda *s: _rng.normal(s) * 0.05)(B, S, D)), 'wq': _w((lambda *s: _rng.normal(s) * 0.05)(D, H * Dh)), 'wk': _w((lambda *s: _rng.normal(s) * 0.05)(D, Dh)), 'wv': _w((lambda *s: _rng.normal(s) * 0.05)(D, Dh)), 'wo': _w((lambda *s: _rng.normal(s) * 0.05)(H * Dh, D))}
    _A_in = _A_setup()

    def _B_setup():
        B, S, D, F = (1, 2048, 576, 4608)
        return {'x': _w((lambda *s: _rng.normal(s) * 0.05)(B, S, D)), 'w_gate': _w((lambda *s: _rng.normal(s) * 0.05)(D, F)), 'w_up': _w((lambda *s: _rng.normal(s) * 0.05)(D, F)), 'w_down': _w((lambda *s: _rng.normal(s) * 0.05)(F, D))}
    _B_in = _B_setup()
    return {'A_x': _A_in['x'], 'A_wq': _A_in['wq'], 'A_wk': _A_in['wk'], 'A_wv': _A_in['wv'], 'A_wo': _A_in['wo'], 'B_x': _B_in['x'], 'B_w_gate': _B_in['w_gate'], 'B_w_up': _B_in['w_up'], 'B_w_down': _B_in['w_down'], 'c': _w((lambda *s: _rng.normal(s) * 0.05)(1, 576) * 8.0), 'w_mod': _w((lambda *s: _rng.normal(s) * 0.05)(576, 6 * 576) * 576 ** (-0.5) * 8.0)}

def reference(A_x, A_wq, A_wk, A_wv, A_wo, B_x, B_w_gate, B_w_up, B_w_down, c, w_mod):

    def _A_ref(x, wq, wk, wv, wo):
        B, S, D = x.shape
        H = 32
        Dh = D // H
        q = (lambda x, *d: x.transpose(*d))((x @ wq).reshape(B, S, H, Dh), 0, 2, 1, 3)
        k = x @ wk
        v = x @ wv
        scores = jnp.einsum('bhqd,bkd->bhqk', q, k) * Dh ** (-0.5)
        p = _softmax(scores, axis=-1)
        o = jnp.einsum('bhqk,bkd->bhqd', p, v)
        return (lambda x, *d: x.transpose(*d))(o, 0, 2, 1, 3).reshape(B, S, H * Dh) @ wo

    def _B_ref(x, w_gate, w_up, w_down):
        g = _silu(x @ w_gate)
        u = x @ w_up
        return g * u @ w_down
    x = A_x
    mod = (_silu(c) @ w_mod).reshape(c.shape[0], 6, 1, -1)
    sa, ca, ga, sb, cb, gb = (mod[:, 0].copy(), mod[:, 1].copy(), mod[:, 2].copy(), mod[:, 3].copy(), mod[:, 4].copy(), mod[:, 5].copy())
    h = _layernorm(x, axis=-1) * (1 + ca) + sa
    x = x + ga * _A_ref(h, A_wq, A_wk, A_wv, A_wo)
    h = _layernorm(x, axis=-1) * (1 + cb) + sb
    x = x + gb * _B_ref(h, B_w_gate, B_w_up, B_w_down)
    return x
```

```python
import functools
import jax
import jax.numpy as jnp
from jax import lax
from jax.experimental import pallas as pl
from jax.experimental.pallas import tpu as pltpu

S = 2048
D = 576
H = 32
DH = 18
F = 4608
EPS = 1e-5
KP = 32
LOG2E = 1.4426950408889634
F32 = jnp.float32
BF16 = jnp.bfloat16


def _dot(a, b):
    return jnp.dot(a, b, preferred_element_type=F32)


def _dot_nt(a, b):
    return lax.dot_general(a, b, (((1,), (1,)), ((), ())), preferred_element_type=F32)


def _ln_t(x):
    m = jnp.mean(x, axis=0, keepdims=True)
    xc = x - m
    v = jnp.mean(xc * xc, axis=0, keepdims=True)
    return xc * lax.rsqrt(v + EPS)


def _rep(col, n):
    return jnp.concatenate([col] * (n // 128), axis=1)


def make_kernel(TQ=512, CK=512, HU=4, FC=512, U=1, TP=512, do_attn=True, do_ffn=True, force_safe=None):
    NQ = S // TQ
    NC = S // CK
    NB = F // (FC * U)

    def kernel(xt_ref, c_ref, wmod_ref, wq_ref, wkT_ref, wvT_ref, wo_ref, wg_hbm, wu_hbm, wdT_hbm,
               o_ref,
               modc_s, wqkv_s, woT_s, qt_s, k_s, vt_s, ot_s, wg_s, wu_s, wdT_s, h2_s, acc_s, flag_s, sems):
        step = pl.program_id(0)

        def w_copies():
            return (pltpu.make_async_copy(wg_hbm, wg_s, sems.at[0]),
                    pltpu.make_async_copy(wu_hbm, wu_s, sems.at[1]),
                    pltpu.make_async_copy(wdT_hbm, wdT_s, sems.at[2]))

        @pl.when(step == 0)
        def _prologue():
            for cp in w_copies():
                cp.start()
            c = c_ref[...].astype(F32)
            sc = c * jax.nn.sigmoid(c)
            sc8 = jnp.broadcast_to(sc, (16, D)).astype(BF16)
            mod = _dot(sc8, wmod_ref[...])[0:1]
            modc_s[...] = jnp.broadcast_to(mod, (128, 6 * D)).T
            wqkv_s[0:D, :] = wq_ref[...].astype(F32).T.astype(BF16)
            zpad = jnp.zeros((KP - DH, D), F32)
            wqkv_s[D:D + KP, :] = jnp.concatenate([wvT_ref[...].astype(F32), zpad], axis=0).astype(BF16)
            wqkv_s[D + KP:D + 2 * KP, :] = jnp.concatenate([wkT_ref[...].astype(F32), zpad], axis=0).astype(BF16)
            woT_s[...] = wo_ref[...].astype(F32).T.astype(BF16)

            qscale = (DH ** -0.5) * LOG2E
            rows = lax.broadcasted_iota(jnp.int32, (KP - 16, TP), 0)

            def tbody(t, carry):
                qmax, kmax, vmax = carry
                t0 = pl.multiple_of(t * TP, TP)
                sa = _rep(modc_s[0:D, :], TP)
                ca1 = _rep(modc_s[D:2 * D, :] + 1.0, TP)
                xs = xt_ref[:, pl.ds(t0, TP)].astype(F32)
                hT = (_ln_t(xs) * ca1 + sa).astype(BF16)
                qkv = _dot(wqkv_s[...], hT)
                kT = qkv[D + KP:D + 2 * KP, :].astype(BF16).astype(F32)
                kmax = jnp.maximum(kmax, jnp.sum(kT * kT, axis=0, keepdims=True))
                kpad = jnp.concatenate([kT, jnp.zeros((128 - KP, TP), F32)], axis=0)
                k_s[pl.ds(t0, TP), :] = kpad.T.astype(BF16)
                for hh in range(H):
                    qh = (qkv[hh * DH:(hh + 1) * DH, :] * qscale).astype(BF16).astype(F32)
                    qmax = jnp.maximum(qmax, jnp.sum(qh * qh, axis=0, keepdims=True))
                    qpad = jnp.concatenate([qh, jnp.zeros((KP - DH, TP), F32)], axis=0)
                    qt_s[hh, :, pl.ds(t0, TP)] = qpad.astype(BF16)
                vt = qkv[D:D + KP, :]
                vmax = jnp.maximum(vmax, jnp.max(jnp.abs(vt), axis=0, keepdims=True))
                vhi = jnp.where(rows == DH - 16, 1.0, vt[16:KP, :])
                vt_s[:, pl.ds(t0, TP)] = jnp.concatenate([vt[0:16, :], vhi], axis=0).astype(BF16)
                return qmax, kmax, vmax
            z = jnp.zeros((1, TP), F32)
            qmax, kmax, vmax = lax.fori_loop(0, S // TP, tbody, (z, z, z))
            bound2 = jnp.max(qmax) * jnp.max(kmax)
            safe = jnp.logical_and(bound2 <= 60.0 * 60.0, jnp.max(vmax) <= 2.0 ** 50)
            flag_s[0] = safe.astype(jnp.int32)

        q0 = pl.multiple_of(step * TQ, TQ)

        def norm(oT):
            return oT[0:DH, :] * (1.0 / oT[DH:DH + 1, :])

        def fast_attn():
            def body(i, carry):
                seq = [(hh, j) for hh in range(HU) for j in range(NC)]
                qTs = [qt_s[HU * i + hh, :, pl.ds(q0, TQ)] for hh in range(HU)]
                oT = [None] * HU
                s_next = _dot(k_s[0:CK, 0:KP], qTs[0])
                for n, (hh, j) in enumerate(seq):
                    s_cur = s_next
                    if n + 1 < len(seq):
                        h2, j2 = seq[n + 1]
                        s_next = _dot(k_s[j2 * CK:(j2 + 1) * CK, 0:KP], qTs[h2])
                    pT = jnp.exp2(s_cur).astype(BF16)
                    pv = _dot(vt_s[:, j * CK:(j + 1) * CK], pT)
                    oT[hh] = pv if oT[hh] is None else oT[hh] + pv
                r0 = pl.multiple_of(i * (HU * DH), 8)
                ot_s[pl.ds(r0, HU * DH), :] = jnp.concatenate([norm(o) for o in oT], axis=0)
                return carry
            lax.fori_loop(0, H // HU, body, 0)

        def safe_attn():
            def body(i, carry):
                outs = []
                for hh in range(4):
                    qT = qt_s[4 * i + hh, :, pl.ds(q0, TQ)]
                    sT = _dot(k_s[:, 0:KP], qT)
                    m = jnp.max(sT, axis=0, keepdims=True)
                    pT = jnp.exp2(sT - m).astype(BF16)
                    outs.append(norm(_dot(vt_s[...], pT)))
                r0 = pl.multiple_of(i * (4 * DH), 8)
                ot_s[pl.ds(r0, 4 * DH), :] = jnp.concatenate(outs, axis=0)
                return carry
            lax.fori_loop(0, H // 4, body, 0)

        if do_attn:
            if force_safe is None:
                pl.when(flag_s[0] == 1)(fast_attn)
                pl.when(flag_s[0] != 1)(safe_attn)
            elif force_safe:
                safe_attn()
            else:
                fast_attn()
            attnT = _dot(woT_s[...], ot_s[...].astype(BF16))
        else:
            attnT = jnp.zeros((D, TQ), F32)

        ga = _rep(modc_s[2 * D:3 * D, :], TQ)
        sb = _rep(modc_s[3 * D:4 * D, :], TQ)
        cb1 = _rep(modc_s[4 * D:5 * D, :] + 1.0, TQ)
        x1 = xt_ref[:, pl.ds(q0, TQ)].astype(F32) + ga * attnT
        ot_s[...] = x1
        h2T = _ln_t(x1) * cb1 + sb
        h2_s[...] = h2T.T.astype(BF16)
        acc_s[...] = jnp.zeros_like(acc_s)

        @pl.when(step == 0)
        def _():
            for cp in w_copies():
                cp.wait()

        if do_ffn:
            def fbody(b, carry):
                h2 = h2_s[...]
                base = b * (FC * U)
                def gu(j):
                    off = pl.multiple_of(base + j * FC, 128)
                    return _dot(h2, wg_s[:, pl.ds(off, FC)]), _dot(h2, wu_s[:, pl.ds(off, FC)])
                acc = None
                nxt = gu(0)
                for j in range(U):
                    g, u = nxt
                    if j + 1 < U:
                        nxt = gu(j + 1)
                    hg = 0.5 * g
                    act = ((hg * u) * (1.0 + jnp.tanh(hg))).astype(BF16)
                    off = pl.multiple_of(base + j * FC, 128)
                    dn = _dot_nt(wdT_s[:, pl.ds(off, FC)], act)
                    acc = dn if acc is None else acc + dn
                acc_s[...] += acc
                return carry
            lax.fori_loop(0, NB, fbody, 0)
        gb = _rep(modc_s[5 * D:6 * D, :], TQ)
        o_ref[...] = (ot_s[...] + gb * acc_s[...]).astype(o_ref.dtype)

    @jax.jit
    def run(A_x, A_wq, A_wk, A_wv, A_wo, B_x, B_w_gate, B_w_up, B_w_down, c, w_mod):
        xT = A_x.reshape(S, D).T
        full = lambda shape: pl.BlockSpec(shape, lambda i: (0,) * len(shape))
        hbm = pl.BlockSpec(memory_space=pl.ANY)
        outT = pl.pallas_call(
            kernel,
            grid=(NQ,),
            in_specs=[full((D, S)), full((1, D)), full((D, 6 * D)), full((D, D)), full((DH, D)), full((DH, D)),
                      full((D, D)), hbm, hbm, hbm],
            out_specs=pl.BlockSpec((D, TQ), lambda i: (0, i)),
            out_shape=jax.ShapeDtypeStruct((D, S), BF16),
            scratch_shapes=[
                pltpu.VMEM((6 * D, 128), F32),
                pltpu.VMEM((D + 2 * KP, D), BF16),
                pltpu.VMEM((D, D), BF16),
                pltpu.VMEM((H, KP, S), BF16),
                pltpu.VMEM((S, 128), BF16),
                pltpu.VMEM((KP, S), BF16),
                pltpu.VMEM((D, TQ), F32),
                pltpu.VMEM((D, F), BF16),
                pltpu.VMEM((D, F), BF16),
                pltpu.VMEM((D, F), BF16),
                pltpu.VMEM((TQ, D), BF16),
                pltpu.VMEM((D, TQ), F32),
                pltpu.SMEM((1,), jnp.int32),
                pltpu.SemaphoreType.DMA((3,)),
            ],
            compiler_params=pltpu.CompilerParams(
                dimension_semantics=("arbitrary",),
                vmem_limit_bytes=100 * 1024 * 1024),
        )(xT, c, w_mod, A_wq, A_wk.T, A_wv.T, A_wo, B_w_gate, B_w_up, B_w_down.T)
        return outT.T.reshape(1, S, D)
    return run


_impl = make_kernel(U=3)


@jax.jit
def pallas_adaLN_cond__grouped_kv_mqa__swiglu_ffn__prompt_kernel(
    A_x: jax.Array,
    A_wq: jax.Array,
    A_wk: jax.Array,
    A_wv: jax.Array,
    A_wo: jax.Array,
    B_x: jax.Array,
    B_w_gate: jax.Array,
    B_w_up: jax.Array,
    B_w_down: jax.Array,
    c: jax.Array,
    w_mod: jax.Array,
):
    return _impl(A_x, A_wq, A_wk, A_wv, A_wo, B_x, B_w_gate, B_w_up, B_w_down, c, w_mod)
```

```python
import jax
import jax.numpy as jnp
from jax import lax
from jax.experimental import pallas as pl
from jax.experimental.pallas import tpu as pltpu

S = 2048
D = 576
H = 32
DH = 18
F = 4608
EPS = 1e-5
KP = 32
KF = 24
LOG2E = 1.4426950408889634
F32 = jnp.float32
BF16 = jnp.bfloat16
L_LO = 2.0 ** -40
L_HI = 2.0 ** 60
MA = 2 * D


def _dot(a, b):
    return jnp.dot(a, b, preferred_element_type=F32)


def _dot_nt(a, b):
    return lax.dot_general(a, b, (((1,), (1,)), ((), ())), preferred_element_type=F32)


def _ln_t(x):
    m = jnp.mean(x, axis=0, keepdims=True)
    xc = x - m
    v = jnp.mean(xc * xc, axis=0, keepdims=True)
    return xc * lax.rsqrt(v + EPS)


def _rep(col, n):
    return jnp.concatenate([col] * (n // 128), axis=1)


def make_kernel(TQ=512, FC=768, U=2, NA=(2, 2, 2, 1), NF=(2, 2, 2, 2), NM=1, reserve=3, tunroll=True,
                clip='aiqk', widef=(0, 0), widea=(0, 0), lagf=False, force_safe=False):
    HU = len(NA)
    NQ = S // TQ
    NG = H // HU
    NFC = F // FC
    NB = F // (FC * U)
    LT = TQ // 128
    UPG_A = sum(NA)
    UPG_F = sum(NF)
    UPG_V = UPG_F - NM
    NIF = UPG_F * NG * LT
    NIV = UPG_V * NG * LT
    IPI = -(-NIV // NB)
    RVT = max(a + f for a, f in zip(NA, NF))
    RV = RVT * 128
    V0 = S - RV
    a_units = [(hh, RVT - NF[hh] - NA[hh] + j) for hh in range(HU) for j in range(NA[hh])]
    f_units = [(hh, RVT - NF[hh] + j) for hh in range(HU) for j in range(NF[hh])]
    KBR = RV // NG
    NZ = 3 + UPG_A * LT
    assert KBR % 16 == 0 and (HU * DH) % 8 == 0

    def kernel(xt_hbm, wmod_hbm, wq_hbm, wo_hbm, c_hbm, wkT_hbm, wvT_hbm, wg_hbm, wu_hbm, wdT_hbm,
               o_ref,
               xt_s, wma_s, wmb_s, wq_s, wo_s,
               modc_s, wqkv_s, woT_s, qt_s, qf_s, k_s, vt_s, vtf_s, kb_s, pa_s, pf_s,
               ot_s, raw_s, ok_s, wg_s, wu_s, wdT_s, h2_s, acc_s,
               c_s, cpad_s, wkT_s, wvT_s, zero_s, sems, wsems):
        step = pl.program_id(0)

        def w_copies():
            cps = []
            for n in range(NFC):
                for m, (src, dst) in enumerate(((wg_hbm, wg_s), (wu_hbm, wu_s), (wdT_hbm, wdT_s))):
                    cps.append(pltpu.make_async_copy(src.at[:, n * FC:(n + 1) * FC], dst.at[n], wsems.at[3 * n + m]))
            return cps

        def x_copy(t):
            t0 = t * TQ if isinstance(t, int) else pl.multiple_of(t * TQ, TQ)
            return pltpu.make_async_copy(xt_hbm.at[:, pl.ds(t0, TQ)], xt_s.at[t], sems.at[8 + t])

        def mxu_unit(t, kt, h, dst, base):
            r0 = V0 + kt * 128
            s = _dot(k_s[r0:r0 + 128, 0:KP], qt_s[t, h])
            for cb in range(LT):
                dst[base + cb] = jnp.exp2(s[:, cb * 128:(cb + 1) * 128]).astype(BF16)

        @pl.when(step == 0)
        def _prologue():
            cp_c = pltpu.make_async_copy(c_hbm, c_s, sems.at[0])
            cp_cp = pltpu.make_async_copy(c_hbm.at[:, 0:384], cpad_s, sems.at[1])
            cp_wk = pltpu.make_async_copy(wkT_hbm, wkT_s, sems.at[2])
            cp_wv = pltpu.make_async_copy(wvT_hbm, wvT_s, sems.at[3])
            cp_wq = pltpu.make_async_copy(wq_hbm, wq_s, sems.at[4])
            cp_ma = pltpu.make_async_copy(wmod_hbm.at[:, 0:MA], wma_s, sems.at[5])
            cp_mb = pltpu.make_async_copy(wmod_hbm.at[:, MA:6 * D], wmb_s, sems.at[6])
            cp_wo = pltpu.make_async_copy(wo_hbm, wo_s, sems.at[7])
            for cp in (cp_wq, cp_c, cp_cp, cp_wk, cp_wv, cp_ma):
                cp.start()
            x_copy(0).start()
            for n in range(NZ):
                zero_s[n] = 0
            cp_wq.wait()
            wqkv_s[0:D, :] = wq_s[...].astype(F32).T.astype(BF16)
            for t in range(1, NQ):
                x_copy(t).start()
            for cp in (cp_c, cp_cp, cp_wk, cp_wv, cp_ma):
                cp.wait()
            cp_mb.start()
            cp_wo.start()
            zpad = jnp.zeros((KP - DH, D), F32)
            wqkv_s[D:D + KP, :] = jnp.concatenate([wvT_s[...].astype(F32), zpad], axis=0).astype(BF16)
            wqkv_s[D + KP:D + 2 * KP, :] = jnp.concatenate([wkT_s[...].astype(F32), zpad], axis=0).astype(BF16)
            c = c_s[...].astype(F32)
            sc = c * jax.nn.sigmoid(c)
            sc8 = jnp.broadcast_to(sc, (16, D)).astype(BF16)
            moda = _dot(sc8, wma_s[...])[0:1]
            modc_s[0:MA, :] = jnp.broadcast_to(moda, (128, MA)).T

            qscale = (DH ** -0.5) * LOG2E
            rows = lax.broadcasted_iota(jnp.int32, (KP - 16, TQ), 0)

            def tbody(t, carry):
                t0 = t * TQ if isinstance(t, int) else pl.multiple_of(t * TQ, TQ)
                if not tunroll:
                    x_copy(t).wait()
                sa = _rep(modc_s[0:D, :], TQ)
                ca1 = _rep(modc_s[D:2 * D, :] + 1.0, TQ)
                xs = xt_s[t].astype(F32)
                hT = (_ln_t(xs) * ca1 + sa).astype(BF16)
                qkv = _dot(wqkv_s[...], hT)
                kT = qkv[D + KP:D + 2 * KP, :]
                kpad = jnp.concatenate([kT, jnp.zeros((128 - KP, TQ), F32)], axis=0)
                k_s[pl.ds(t0, TQ), :] = kpad.T.astype(BF16)
                for hh in range(H):
                    qh = qkv[hh * DH:(hh + 1) * DH, :] * qscale
                    qpad = jnp.concatenate([qh, jnp.zeros((KP - DH, TQ), F32)], axis=0).astype(BF16)
                    qt_s[t, hh] = qpad
                    qpf = qpad.astype(F32)
                    for cb in range(LT):
                        qf_s[hh, t * LT + cb, 0:KF, :] = qpf[0:KF, cb * 128:(cb + 1) * 128]
                vt = qkv[D:D + KP, :]
                vhi = jnp.where(rows == DH - 16, 1.0, vt[16:KP, :])
                vb = jnp.concatenate([vt[0:16, :], vhi], axis=0).astype(BF16)
                vt_s[:, pl.ds(t0, TQ)] = vb
                vtf_s[:, pl.ds(t0, TQ)] = vb.astype(F32)[0:KF]
                return carry
            if tunroll:
                x_copy(0).wait()
                tbody(0, 0)
                for t in range(1, NQ):
                    x_copy(t).wait()
                for t in range(1, NQ):
                    tbody(t, 0)
            else:
                lax.fori_loop(0, NQ, tbody, 0)
            for cp in w_copies():
                cp.start()

            def pbody(g, carry):
                for j, (hh, kt) in enumerate(f_units):
                    mxu_unit(0, kt, HU * g + hh, pf_s, (UPG_F * g + j) * LT)
                r0 = pl.multiple_of(V0 + g * KBR, 16)
                kf = k_s[pl.ds(r0, KBR), :].astype(F32)
                for d in range(DH):
                    kb_s[pl.ds(g * (KBR // 8), KBR // 8), d] = jnp.broadcast_to(
                        kf[:, d:d + 1], (KBR, 128)).reshape(KBR // 8, 8, 128)
                return carry
            lax.fori_loop(0, NG, pbody, 0)
            cp_mb.wait()
            cp_wo.wait()
            for j, (hh, kt) in enumerate(a_units):
                mxu_unit(0, kt, hh, pa_s, j * LT)
            modb = _dot(sc8, wmb_s[...])[0:1]
            modc_s[MA:6 * D, :] = jnp.broadcast_to(modb, (128, 6 * D - MA)).T
            woT_s[...] = wo_s[...].astype(F32).T.astype(BF16)

        tn = jnp.minimum(step + 1, NQ - 1)
        never = [jnp.full((8, 128), zero_s[n], jnp.int32) != 0 for n in range(3)]

        def clamp(x, hi, tag="a"):
            return jnp.clip(x, 0, hi) if tag in clip else x

        def vpu_items(items, lag, wide=()):
            tasks = [(it, rb) for it in range(len(items)) for rb in range(16)]
            qbs = {}
            prev, prev2, done = [], [], []
            n = stp = 0
            while n < len(tasks):
                w = min(3 if stp in wide else 2, len(tasks) - n)
                cur = []
                for j in range(w):
                    it, rb = tasks[n + j]
                    qfn, kb0, store = items[it]
                    if it not in qbs:
                        qbs[it] = qfn()
                    qb = qbs[it]
                    acc = kb_s[kb0 + rb, 0] * qb[0]
                    if lag and j < len(prev2):
                        acc = jnp.where(never[1], prev2[j][1], acc)
                    if j == 0 and len(prev) > w:
                        acc = jnp.where(never[2], prev[w][0], acc)
                    if prev:
                        acc = jnp.where(never[0], prev[j % len(prev)][0], acc)
                    for d in range(1, DH):
                        acc = acc + kb_s[kb0 + rb, d] * qb[d]
                    cur.append((acc, jnp.exp2(acc)))
                    done.append(cur[-1][1])
                    if len(done) == 2:
                        store((rb - 1) * 8, jnp.concatenate(done, axis=0).astype(BF16))
                        done = []
                prev2, prev = prev, cur
                n += w
                stp += 1

        def bcast_q(h, lt):
            q = qf_s[h, lt, 0:KF, :]
            return [jnp.broadcast_to(q[d:d + 1, :], (8, 128)) for d in range(DH)]

        def norm(oT):
            l = oT[DH:DH + 1, :]
            return oT[0:DH, :] * (1.0 / l), l

        ok_s[...] = jnp.ones_like(ok_s)
        raw_s[...] = jnp.ones_like(raw_s)

        def finish(i):
            outs = []
            ok = ok_s[...]
            for hh in range(HU):
                o, l = norm(raw_s[hh])
                outs.append(o)
                fin = jnp.min(jnp.where(jnp.abs(o) <= 3.0e38, 1.0, 0.0), axis=0, keepdims=True)
                good = jnp.logical_and(l >= L_LO, l <= L_HI)
                ok = jnp.where(good, ok * fin, 0.0)
            ok_s[...] = ok
            r0 = pl.multiple_of(i * (HU * DH), 8)
            ot_s[pl.ds(r0, HU * DH), :] = jnp.concatenate(outs, axis=0)

        def abody(i, carry):
            finish(jnp.maximum(i - 1, 0))
            qTs = [qt_s[step, HU * i + hh] for hh in range(HU)]
            oT = [None] * HU

            def add(hh, v):
                oT[hh] = v if oT[hh] is None else oT[hh] + v

            def unit_pv(kind, j):
                hh, kt = (a_units if kind == "a" else f_units)[j]
                r0 = V0 + kt * 128
                if kind == "a":
                    p = jnp.concatenate([pa_s[j * LT + cb] for cb in range(LT)], axis=1)
                else:
                    p = jnp.concatenate([pf_s[(UPG_F * i + j) * LT + cb] for cb in range(LT)], axis=1)
                add(hh, _dot(vt_s[:, r0:r0 + 128], p)[0:KF])

            units = [("a", j) for j in range(UPG_A)] + [("f", j) for j in range(UPG_F)]
            ready = []

            def own_pv(n):
                tiles = [ready.pop(0) for _ in range(n)]
                if n == 2 and tiles[0][0] == tiles[1][0]:
                    hh, r0, _ = tiles[0]
                    add(hh, _dot(vtf_s[:, r0:r0 + 256], jnp.concatenate([tiles[0][2], tiles[1][2]], axis=0)))
                else:
                    for hh, r0, p in tiles:
                        add(hh, _dot(vtf_s[:, r0:r0 + 128], p))

            for hh in range(HU):
                rows = 256 - 16 * (NA[hh] + NF[hh])
                buf = None
                r0 = 0
                for k in range(8):
                    p = jnp.exp2(_dot(k_s[k * rows:(k + 1) * rows, 0:KP], qTs[hh]))
                    n_own = min(2, len(ready))
                    for _ in range(min(2 - n_own, max(len(units) - reserve, 0))):
                        unit_pv(*units.pop(0))
                    own_pv(n_own)
                    buf = p if buf is None else jnp.concatenate([buf, p], axis=0)
                    while buf is not None and buf.shape[0] >= 128:
                        ready.append((hh, r0, buf[0:128]))
                        r0 += 128
                        buf = buf[128:] if buf.shape[0] > 128 else None
                assert buf is None
            for u in units:
                unit_pv(*u)
            while ready:
                own_pv(min(2, len(ready)))

            last = i == NG - 1
            gn = jnp.where(last, 0, i + 1)
            tsn = jnp.where(last, tn, step)
            items = []
            for hh in range(HU):
                for cb in range(LT):
                    cache = {}

                    def qfn(hh=hh, cb=cb, cache=cache):
                        if "q" not in cache:
                            cache["q"] = bcast_q(HU * gn + hh, tsn * LT + cb)
                        return cache["q"]
                    for j, (h2, kt) in enumerate(a_units):
                        if h2 != hh:
                            continue

                        def store(rr, val, j=j, cb=cb):
                            pa_s[j * LT + cb, rr:rr + 16, :] = val
                        kb0 = clamp(kt + zero_s[3 + j * LT + cb], RVT - 1) * 16
                        items.append((qfn, kb0, store))
            vpu_items(items, True, set(range(*widea)))
            for hh in range(HU):
                raw_s[hh] = oT[hh]
            return carry
        lax.fori_loop(0, NG, abody, 0)
        finish(NG - 1)

        def safe_attn():
            def body(i, carry):
                def hbody(hh, c2):
                    sT = _dot(k_s[:, 0:KP], qt_s[step, HU * i + hh])
                    m = jnp.max(sT, axis=0, keepdims=True)
                    raw_s[hh] = _dot(vtf_s[...], jnp.exp2(sT - m))
                    return c2
                lax.fori_loop(0, HU, hbody, 0)
                r0 = pl.multiple_of(i * (HU * DH), 8)
                ot_s[pl.ds(r0, HU * DH), :] = jnp.concatenate([norm(raw_s[hh])[0] for hh in range(HU)], axis=0)
                return carry
            lax.fori_loop(0, NG, body, 0)

        if force_safe:
            safe_attn()
        else:
            pl.when(jnp.min(ok_s[...]) < 0.5)(safe_attn)

        attnT = _dot(woT_s[...], ot_s[...].astype(BF16))
        ga = _rep(modc_s[2 * D:3 * D, :], TQ)
        sb = _rep(modc_s[3 * D:4 * D, :], TQ)
        cb1 = _rep(modc_s[4 * D:5 * D, :] + 1.0, TQ)
        x1 = xt_s[step].astype(F32) + ga * attnT
        acc_s[...] = x1
        h2T = _ln_t(x1) * cb1 + sb
        h2_s[...] = h2T.T.astype(BF16)
        for g in range(NG):
            for j in range(UPG_V, UPG_F):
                hh, kt = f_units[j]
                mxu_unit(tn, kt, HU * g + hh, pf_s, (UPG_F * g + j) * LT)

        @pl.when(step == 0)
        def _():
            for cp in w_copies():
                cp.wait()

        def fbody(b, carry):
            h2 = h2_s[...]

            def gu(j):
                return _dot(h2, wg_s[b * U + j]), _dot(h2, wu_s[b * U + j])
            acc = None
            nxt = gu(0)
            for j in range(U):
                g, u = nxt
                if j + 1 < U:
                    nxt = gu(j + 1)
                hg = 0.5 * g
                act = ((hg * u) * (1.0 + jnp.tanh(hg))).astype(BF16)
                dn = _dot_nt(wdT_s[b * U + j], act)
                acc = dn if acc is None else acc + dn
            gb = _rep(modc_s[5 * D:6 * D, :], TQ)
            acc_s[...] += gb * acc
            items = []
            for jj in range(IPI):
                iv = jnp.minimum(b * IPI + jj, NIV - 1)
                un = iv // LT
                cb = iv - un * LT
                g = un // UPG_V
                j = un - g * UPG_V
                it = clamp((g * UPG_F + j) * LT + cb, NIF - 1, 'i')
                hh = sum(jnp.where(j == n, fu[0], 0) for n, fu in enumerate(f_units))
                kt = sum(jnp.where(j == n, fu[1], 0) for n, fu in enumerate(f_units))

                def qfn(h=clamp(HU * g + hh, H - 1, 'q'), lt=clamp(tn * LT + cb, S // 128 - 1, 'q')):
                    return bcast_q(h, lt)

                def store(rr, val, it=it):
                    pf_s[it, rr:rr + 16, :] = val
                items.append((qfn, clamp(kt, RVT - 1, 'k') * 16, store))
            vpu_items(items, lagf, set(range(*widef)))
            return carry
        lax.fori_loop(0, NB, fbody, 0)
        o_ref[...] = acc_s[...].astype(o_ref.dtype)

    @jax.jit
    def run(A_x, A_wq, A_wk, A_wv, A_wo, B_x, B_w_gate, B_w_up, B_w_down, c, w_mod):
        xT = A_x.reshape(S, D).T
        hbm = pl.BlockSpec(memory_space=pl.ANY)
        outT = pl.pallas_call(
            kernel,
            grid=(NQ,),
            in_specs=[hbm] * 10,
            out_specs=pl.BlockSpec((D, TQ), lambda i: (0, i)),
            out_shape=jax.ShapeDtypeStruct((D, S), BF16),
            scratch_shapes=[
                pltpu.VMEM((NQ, D, TQ), BF16),
                pltpu.VMEM((D, MA), BF16),
                pltpu.VMEM((D, 6 * D - MA), BF16),
                pltpu.VMEM((D, D), BF16),
                pltpu.VMEM((D, D), BF16),
                pltpu.VMEM((6 * D, 128), F32),
                pltpu.VMEM((D + 2 * KP, D), BF16),
                pltpu.VMEM((D, D), BF16),
                pltpu.VMEM((NQ, H, KP, TQ), BF16),
                pltpu.VMEM((H, S // 128, KP, 128), F32),
                pltpu.VMEM((S, 128), BF16),
                pltpu.VMEM((KP, S), BF16),
                pltpu.VMEM((KF, S), F32),
                pltpu.VMEM((RV // 8, DH, 8, 128), F32),
                pltpu.VMEM((UPG_A * LT, 128, 128), BF16),
                pltpu.VMEM((NIF, 128, 128), BF16),
                pltpu.VMEM((D, TQ), F32),
                pltpu.VMEM((HU, KF, TQ), F32),
                pltpu.VMEM((8, TQ), F32),
                pltpu.VMEM((NFC, D, FC), BF16),
                pltpu.VMEM((NFC, D, FC), BF16),
                pltpu.VMEM((NFC, D, FC), BF16),
                pltpu.VMEM((TQ, D), BF16),
                pltpu.VMEM((D, TQ), F32),
                pltpu.VMEM((1, D), BF16),
                pltpu.VMEM((1, 384), BF16),
                pltpu.VMEM((DH, D), BF16),
                pltpu.VMEM((DH, D), BF16),
                pltpu.SMEM((NZ,), jnp.int32),
                pltpu.SemaphoreType.DMA((8 + NQ,)),
                pltpu.SemaphoreType.DMA((3 * NFC,)),
            ],
            compiler_params=pltpu.CompilerParams(
                dimension_semantics=("arbitrary",),
                vmem_limit_bytes=110 * 1024 * 1024),
        )(xT, w_mod, A_wq, A_wo, c, A_wk.T, A_wv.T, B_w_gate, B_w_up, B_w_down.T)
        return outT.T.reshape(1, S, D)
    return run


_impl = make_kernel()


@jax.jit
def pallas_adaLN_cond__grouped_kv_mqa__swiglu_ffn__prompt_kernel(
    A_x: jax.Array,
    A_wq: jax.Array,
    A_wk: jax.Array,
    A_wv: jax.Array,
    A_wo: jax.Array,
    B_x: jax.Array,
    B_w_gate: jax.Array,
    B_w_up: jax.Array,
    B_w_down: jax.Array,
    c: jax.Array,
    w_mod: jax.Array,
):
    return _impl(A_x, A_wq, A_wk, A_wv, A_wo, B_x, B_w_gate, B_w_up, B_w_down, c, w_mod)
```

```python
import jax
import jax.numpy as jnp
from jax import lax
from jax.experimental import pallas as pl
from jax.experimental.pallas import tpu as pltpu

S = 2048
D = 576
H = 32
DH = 18
F = 4608
EPS = 1e-5
KP = 32
KF = 24
LOG2E = 1.4426950408889634
F32 = jnp.float32
BF16 = jnp.bfloat16
L_LO = 2.0 ** -40
L_HI = 2.0 ** 60
MA = 2 * D

TQ = 512
NQ = S // TQ
LT = TQ // 128
FC = 768
U = 2
NFC = F // FC
NB = F // (FC * U)

NA = (2, 2, 1, 2)
NF = (2, 2, 2, 2)
HU = len(NA)
NG = H // HU
UPG_A = sum(NA)
UPG_F = sum(NF)
NIF = UPG_F * NG * LT
RVT = max(a + f for a, f in zip(NA, NF))
RV = RVT * 128
V0 = S - RV
A_UNITS = [(hh, RVT - NF[hh] - NA[hh] + j) for hh in range(HU) for j in range(NA[hh])]
F_UNITS = [(hh, RVT - NF[hh] + j) for hh in range(HU) for j in range(NF[hh])]
V_LIST = [(g, j) for g in range(NG) for j in range(UPG_F) if j < UPG_F - 1 or g < 3]
M_LIST = [(g, j) for g in range(NG) for j in range(UPG_F) if (g, j) not in V_LIST]
NIV = len(V_LIST) * LT
IPI = -(-NIV // NB)
RESERVE = 4
KBR = RV // NG
NZ = 3 + UPG_A * LT
TABLE = []
for _n in range(NB * IPI):
    _un, _cb = divmod(min(_n, NIV - 1), LT)
    _g, _j = V_LIST[_un]
    TABLE += [(_g * UPG_F + _j) * LT + _cb, HU * _g + F_UNITS[_j][0], _cb, F_UNITS[_j][1]]


def _dot(a, b):
    return jnp.dot(a, b, preferred_element_type=F32)


def _dot_nt(a, b):
    return lax.dot_general(a, b, (((1,), (1,)), ((), ())), preferred_element_type=F32)


def _ln_t(x):
    m = jnp.mean(x, axis=0, keepdims=True)
    xc = x - m
    v = jnp.mean(xc * xc, axis=0, keepdims=True)
    return xc * lax.rsqrt(v + EPS)


def _rep(col, n):
    return jnp.concatenate([col] * (n // 128), axis=1)


def _kernel(xt_hbm, wmod_hbm, wq_hbm, wo_hbm, c_hbm, wkT_hbm, wvT_hbm, wg_hbm, wu_hbm, wdT_hbm,
            o_ref,
            xt_s, wma_s, wmb_s, wq_s, wo_s,
            modc_s, wqkv_s, woT_s, qt_s, qf_s, k_s, vtf_s, kb_s, pa_s, pf_s,
            ot_s, raw_s, ok_s, wg_s, wu_s, wdT_s, h2_s, acc_s,
            c_s, cpad_s, wkT_s, wvT_s, zero_s, tab_s, sems, wsems):
    step = pl.program_id(0)

    def w_copies():
        cps = []
        for n in range(NFC):
            for m, (src, dst) in enumerate(((wg_hbm, wg_s), (wu_hbm, wu_s), (wdT_hbm, wdT_s))):
                cps.append(pltpu.make_async_copy(src.at[:, n * FC:(n + 1) * FC], dst.at[n], wsems.at[3 * n + m]))
        return cps

    def x_copy(t):
        return pltpu.make_async_copy(xt_hbm.at[:, t * TQ:(t + 1) * TQ], xt_s.at[t], sems.at[8 + t])

    def mxu_unit(t, kt, h, dst, base):
        r0 = V0 + kt * 128
        s = _dot(k_s[r0:r0 + 128, 0:KP], qt_s[t, h])
        for cb in range(LT):
            dst[base + cb] = jnp.exp2(s[:, cb * 128:(cb + 1) * 128])

    @pl.when(step == 0)
    def _prologue():
        cp_c = pltpu.make_async_copy(c_hbm, c_s, sems.at[0])
        cp_cp = pltpu.make_async_copy(c_hbm.at[:, 0:384], cpad_s, sems.at[1])
        cp_wk = pltpu.make_async_copy(wkT_hbm, wkT_s, sems.at[2])
        cp_wv = pltpu.make_async_copy(wvT_hbm, wvT_s, sems.at[3])
        cp_wq = pltpu.make_async_copy(wq_hbm, wq_s, sems.at[4])
        cp_ma = pltpu.make_async_copy(wmod_hbm.at[:, 0:MA], wma_s, sems.at[5])
        cp_mb = pltpu.make_async_copy(wmod_hbm.at[:, MA:6 * D], wmb_s, sems.at[6])
        cp_wo = pltpu.make_async_copy(wo_hbm, wo_s, sems.at[7])
        for cp in (cp_wq, cp_c, cp_cp, cp_wk, cp_wv, cp_ma):
            cp.start()
        x_copy(0).start()
        for n in range(NZ):
            zero_s[n] = 0
        for n, v in enumerate(TABLE):
            tab_s[n] = v
        cp_wq.wait()
        wqkv_s[0:D, :] = wq_s[...].astype(F32).T.astype(BF16)
        for cp in (cp_c, cp_cp, cp_wk, cp_wv, cp_ma):
            cp.wait()
        for t in range(1, NQ):
            x_copy(t).start()
        zpad = jnp.zeros((KP - DH, D), F32)
        wqkv_s[D:D + KP, :] = jnp.concatenate([wvT_s[...].astype(F32), zpad], axis=0).astype(BF16)
        wqkv_s[D + KP:D + 2 * KP, :] = jnp.concatenate([wkT_s[...].astype(F32), zpad], axis=0).astype(BF16)
        c = c_s[...].astype(F32)
        sc = c * jax.nn.sigmoid(c)
        sc8 = jnp.broadcast_to(sc, (16, D)).astype(BF16)
        moda = _dot(sc8, wma_s[...])[0:1]
        modc_s[0:MA, :] = jnp.broadcast_to(moda, (128, MA)).T

        qscale = (DH ** -0.5) * LOG2E
        rows = lax.broadcasted_iota(jnp.int32, (KP - 16, TQ), 0)

        def project(t):
            t0 = t * TQ
            sa = _rep(modc_s[0:D, :], TQ)
            ca1 = _rep(modc_s[D:2 * D, :] + 1.0, TQ)
            hT = (_ln_t(xt_s[t].astype(F32)) * ca1 + sa).astype(BF16)
            qkv = _dot(wqkv_s[...], hT)
            kT = qkv[D + KP:D + 2 * KP, :]
            kpad = jnp.concatenate([kT, jnp.zeros((128 - KP, TQ), F32)], axis=0)
            k_s[t0:t0 + TQ, :] = kpad.T.astype(BF16)
            for hh in range(H):
                qh = qkv[hh * DH:(hh + 1) * DH, :] * qscale
                qpad = jnp.concatenate([qh, jnp.zeros((KP - DH, TQ), F32)], axis=0).astype(BF16)
                qt_s[t, hh] = qpad
                qpf = qpad.astype(F32)
                for cb in range(LT):
                    qf_s[hh, t * LT + cb, 0:KF, :] = qpf[0:KF, cb * 128:(cb + 1) * 128]
            vt = qkv[D:D + KP, :]
            vhi = jnp.where(rows == DH - 16, 1.0, vt[16:KP, :])
            vb = jnp.concatenate([vt[0:16, :], vhi], axis=0).astype(BF16)
            vtf_s[:, t0:t0 + TQ] = vb.astype(F32)[0:KF]

        x_copy(0).wait()
        project(0)
        for t in range(1, NQ):
            x_copy(t).wait()
        cp_mb.start()
        cp_wo.start()
        for t in range(1, NQ):
            project(t)

        def pbody(g, carry):
            for j, (hh, kt) in enumerate(F_UNITS):
                mxu_unit(0, kt, HU * g + hh, pf_s, (UPG_F * g + j) * LT)
            r0 = V0 + g * KBR if isinstance(g, int) else pl.multiple_of(V0 + g * KBR, 16)
            kf = k_s[pl.ds(r0, KBR), :].astype(F32)
            for d in range(DH):
                kb_s[pl.ds(g * (KBR // 16), KBR // 16), :, d] = jnp.broadcast_to(
                    kf[:, d:d + 1], (KBR, 128)).reshape(KBR // 16, 2, 8, 128)
            return carry
        lax.fori_loop(0, NG - 1, pbody, 0)
        cp_mb.wait()
        cp_wo.wait()
        for cp in w_copies():
            cp.start()
        modb = _dot(sc8, wmb_s[...])[0:1]
        modc_s[MA:6 * D, :] = jnp.broadcast_to(modb, (128, 6 * D - MA)).T
        woT_s[...] = wo_s[...].astype(F32).T.astype(BF16)
        pbody(NG - 1, 0)
        for j, (hh, kt) in enumerate(A_UNITS):
            mxu_unit(0, kt, hh, pa_s, j * LT)

    tn = jnp.minimum(step + 1, NQ - 1)
    never = [jnp.full((2, 8, 128), zero_s[n], jnp.int32) != 0 for n in range(2)]

    def clamp(x, hi):
        return jnp.clip(x, 0, hi)

    def vpu_items(items, lag, dc):
        hist = []
        for qfn, kb0, store in items:
            qb = qfn()
            for rb in range(8):
                acc = None
                for d0 in range(0, DH, dc):
                    prod = kb_s[kb0 + rb, :, d0:d0 + dc] * qb[None, d0:d0 + dc]
                    if acc is None:
                        acc = prod[:, 0]
                        prod = prod[:, 1:]
                        if lag and len(hist) >= lag:
                            acc = jnp.where(never[1], hist[-lag][1], acc)
                        if hist:
                            acc = jnp.where(never[0], hist[-1][0], acc)
                    acc = jnp.sum(jnp.concatenate([acc[:, None], prod], axis=1), axis=1)
                hist.append((acc, jnp.exp2(acc)))
                store(rb * 16, hist[-1][1].reshape(16, 128))

    def bcast_q(h, lt):
        q = qf_s[h, lt, 0:KF, :]
        return jnp.stack([jnp.broadcast_to(q[d:d + 1, :], (8, 128)) for d in range(DH)], axis=0)

    def norm(oT):
        l = oT[DH:DH + 1, :]
        return oT[0:DH, :] * (1.0 / l), l

    ok_s[...] = jnp.ones_like(ok_s)
    raw_s[...] = jnp.ones_like(raw_s)

    def finish(i):
        outs = []
        ok = ok_s[...]
        for hh in range(HU):
            o, l = norm(raw_s[hh])
            outs.append(o)
            fin = jnp.min(jnp.where(jnp.abs(o) <= 3.0e38, 1.0, 0.0), axis=0, keepdims=True)
            good = jnp.logical_and(l >= L_LO, l <= L_HI)
            ok = jnp.where(good, ok * fin, 0.0)
        ok_s[...] = ok
        r0 = pl.multiple_of(i * (HU * DH), 8)
        ot_s[pl.ds(r0, HU * DH), :] = jnp.concatenate(outs, axis=0)

    def abody(i, carry):
        finish(jnp.maximum(i - 1, 0))
        qTs = [qt_s[step, HU * i + hh] for hh in range(HU)]
        oT = [None] * HU

        def add(hh, v):
            oT[hh] = v if oT[hh] is None else oT[hh] + v

        def unit_tile(kind, j):
            hh, kt = (A_UNITS if kind == "a" else F_UNITS)[j]

            def get():
                if kind == "a":
                    return jnp.concatenate([pa_s[j * LT + cb] for cb in range(LT)], axis=1)
                return jnp.concatenate([pf_s[(UPG_F * i + j) * LT + cb] for cb in range(LT)], axis=1)
            return (hh, V0 + kt * 128, get)

        def pv(tiles):
            if len(tiles) == 2 and tiles[0][0] == tiles[1][0]:
                v = jnp.concatenate([vtf_s[:, t[1]:t[1] + 128] for t in tiles], axis=1)
                add(tiles[0][0], _dot(v, jnp.concatenate([t[2]() for t in tiles], axis=0)))
            else:
                for hh, r0, get in tiles:
                    add(hh, _dot(vtf_s[:, r0:r0 + 128], get()))

        units = [unit_tile("a", j) for j in range(UPG_A)] + [unit_tile("f", j) for j in range(UPG_F)]
        tail = units[len(units) - RESERVE:]
        units = units[:len(units) - RESERVE]
        ready = []

        def unit_pair():
            for n, u in enumerate(units):
                for m in range(n + 1, len(units)):
                    if units[m][0] == u[0]:
                        b = units.pop(m)
                        return [units.pop(n), b]
            return None

        for hh in range(HU):
            rows = 256 - 16 * (NA[hh] + NF[hh])
            buf = None
            r0 = 0
            for k in range(8):
                p = jnp.exp2(_dot(k_s[k * rows:(k + 1) * rows, 0:KP], qTs[hh]))
                if len(ready) >= 2:
                    pv([ready.pop(0), ready.pop(0)])
                elif ready:
                    pv(([units.pop(0)] if units else []) + [ready.pop(0)])
                else:
                    pv(unit_pair())
                buf = p if buf is None else jnp.concatenate([buf, p], axis=0)
                while buf is not None and buf.shape[0] >= 128:
                    ready.append((hh, r0, lambda v=buf[0:128]: v))
                    r0 += 128
                    buf = buf[128:] if buf.shape[0] > 128 else None
            assert buf is None
        while len(ready) > 2:
            pv([ready.pop(0), ready.pop(0)])
        units.extend(tail)
        while units:
            up = unit_pair()
            pv(up if up is not None else [units.pop(0)])
        pv(ready)

        last = i == NG - 1
        gn = jnp.where(last, 0, i + 1)
        tsn = jnp.where(last, tn, step)
        cache = {}
        items = []
        for j, (hh, kt) in enumerate(A_UNITS):
            for cb in range(LT):
                def qfn(hh=hh, cb=cb):
                    if (hh, cb) not in cache:
                        cache[(hh, cb)] = bcast_q(HU * gn + hh, tsn * LT + cb)
                    return cache[(hh, cb)]

                def store(rr, val, j=j, cb=cb):
                    pa_s[j * LT + cb, rr:rr + 16, :] = val
                kb0 = clamp(kt + zero_s[3 + j * LT + cb], RVT - 1) * 8
                items.append(((hh, cb, j), (qfn, kb0, store)))
        items.sort(key=lambda x: x[0])
        vpu_items([it for _, it in items], 3, 2)
        for hh in range(HU):
            raw_s[hh] = oT[hh]
        return carry
    lax.fori_loop(0, NG, abody, 0)

    def safe_attn():
        def body(i, carry):
            def hbody(hh, c2):
                sT = _dot(k_s[:, 0:KP], qt_s[step, HU * i + hh])
                m = jnp.max(sT, axis=0, keepdims=True)
                raw_s[hh] = _dot(vtf_s[...], jnp.exp2(sT - m))
                return c2
            lax.fori_loop(0, HU, hbody, 0)
            r0 = pl.multiple_of(i * (HU * DH), 8)
            ot_s[pl.ds(r0, HU * DH), :] = jnp.concatenate([norm(raw_s[hh])[0] for hh in range(HU)], axis=0)
            return carry
        lax.fori_loop(0, NG, body, 0)

    def mid():
        attnT = _dot(woT_s[...], ot_s[...].astype(BF16))
        ga = _rep(modc_s[2 * D:3 * D, :], TQ)
        sb = _rep(modc_s[3 * D:4 * D, :], TQ)
        cb1 = _rep(modc_s[4 * D:5 * D, :] + 1.0, TQ)
        x1 = xt_s[step].astype(F32) + ga * attnT
        acc_s[...] = x1
        h2T = _ln_t(x1) * cb1 + sb
        h2_s[...] = h2T.T.astype(BF16)
        for g, j in M_LIST:
            hh, kt = F_UNITS[j]
            mxu_unit(tn, kt, HU * g + hh, pf_s, (UPG_F * g + j) * LT)

    def mbody(c):
        pl.when(c == 1)(safe_attn)
        finish(NG - 1)
        bad = jnp.min(ok_s[...]) < 0.5
        mid()
        return jnp.where(jnp.logical_and(c == 0, bad), 1, 2)
    lax.while_loop(lambda c: c < 2, mbody, jnp.int32(0))

    @pl.when(step == 0)
    def _():
        for cp in w_copies():
            cp.wait()

    def fbody(b, carry):
        h2 = h2_s[...]

        def gu(j):
            return _dot(h2, wg_s[b * U + j]), _dot(h2, wu_s[b * U + j])
        acc = None
        nxt = gu(0)
        for j in range(U):
            g, u = nxt
            if j + 1 < U:
                nxt = gu(j + 1)
            hg = 0.5 * g
            act = ((hg * u) * (1.0 + jnp.tanh(hg))).astype(BF16)
            dn = _dot_nt(wdT_s[b * U + j], act)
            acc = dn if acc is None else acc + dn
        gb = _rep(modc_s[5 * D:6 * D, :], TQ)
        acc_s[...] += gb * acc
        items = []
        for jj in range(IPI):
            e = (b * IPI + jj) * 4
            it = clamp(tab_s[e], NIF - 1)

            def qfn(h=clamp(tab_s[e + 1], H - 1), lt=clamp(tn * LT + tab_s[e + 2], S // 128 - 1)):
                return bcast_q(h, lt)

            def store(rr, val, it=it):
                pf_s[it, rr:rr + 16, :] = val
            items.append((qfn, clamp(tab_s[e + 3], RVT - 1) * 8, store))
        vpu_items(items, 0, DH)
        return carry
    lax.fori_loop(0, NB, fbody, 0)
    o_ref[...] = acc_s[...].astype(o_ref.dtype)


@jax.jit
def pallas_adaLN_cond__grouped_kv_mqa__swiglu_ffn__prompt_kernel(
    A_x: jax.Array,
    A_wq: jax.Array,
    A_wk: jax.Array,
    A_wv: jax.Array,
    A_wo: jax.Array,
    B_x: jax.Array,
    B_w_gate: jax.Array,
    B_w_up: jax.Array,
    B_w_down: jax.Array,
    c: jax.Array,
    w_mod: jax.Array,
):
    del B_x
    xT = A_x.reshape(S, D).T
    hbm = pl.BlockSpec(memory_space=pl.ANY)
    outT = pl.pallas_call(
        _kernel,
        grid=(NQ,),
        in_specs=[hbm] * 10,
        out_specs=pl.BlockSpec((D, TQ), lambda i: (0, i)),
        out_shape=jax.ShapeDtypeStruct((D, S), BF16),
        scratch_shapes=[
            pltpu.VMEM((NQ, D, TQ), BF16),
            pltpu.VMEM((D, MA), BF16),
            pltpu.VMEM((D, 6 * D - MA), BF16),
            pltpu.VMEM((D, D), BF16),
            pltpu.VMEM((D, D), BF16),
            pltpu.VMEM((6 * D, 128), F32),
            pltpu.VMEM((D + 2 * KP, D), BF16),
            pltpu.VMEM((D, D), BF16),
            pltpu.VMEM((NQ, H, KP, TQ), BF16),
            pltpu.VMEM((H, S // 128, KP, 128), F32),
            pltpu.VMEM((S, 128), BF16),
            pltpu.VMEM((KF, S), F32),
            pltpu.VMEM((RV // 16, 2, DH, 8, 128), F32),
            pltpu.VMEM((UPG_A * LT, 128, 128), F32),
            pltpu.VMEM((NIF, 128, 128), F32),
            pltpu.VMEM((D, TQ), F32),
            pltpu.VMEM((HU, KF, TQ), F32),
            pltpu.VMEM((8, TQ), F32),
            pltpu.VMEM((NFC, D, FC), BF16),
            pltpu.VMEM((NFC, D, FC), BF16),
            pltpu.VMEM((NFC, D, FC), BF16),
            pltpu.VMEM((TQ, D), BF16),
            pltpu.VMEM((D, TQ), F32),
            pltpu.VMEM((1, D), BF16),
            pltpu.VMEM((1, 384), BF16),
            pltpu.VMEM((DH, D), BF16),
            pltpu.VMEM((DH, D), BF16),
            pltpu.SMEM((NZ,), jnp.int32),
            pltpu.SMEM((len(TABLE),), jnp.int32),
            pltpu.SemaphoreType.DMA((8 + NQ,)),
            pltpu.SemaphoreType.DMA((3 * NFC,)),
        ],
        compiler_params=pltpu.CompilerParams(
            dimension_semantics=("arbitrary",),
            vmem_limit_bytes=110 * 1024 * 1024),
    )(xT, w_mod, A_wq, A_wo, c, A_wk.T, A_wv.T, B_w_gate, B_w_up, B_w_down.T)
    return outT.T.reshape(1, S, D)
```

```python
import jax
import jax.numpy as jnp
from jax import lax
from jax.experimental import pallas as pl
from jax.experimental.pallas import tpu as pltpu

S = 2048
D = 576
H = 32
DH = 18
F = 4608
EPS = 1e-5
KP = 32
KF = 24
LOG2E = 1.4426950408889634
F32 = jnp.float32
BF16 = jnp.bfloat16
L_LO = 1.0
L_HI = 2.0 ** 60
V_HI = 2.0 ** 60
MA = 2 * D

TQ = 512
NQ = S // TQ
LT = TQ // 128
FC = 768
U = 2
NFC = F // FC
NB = F // (FC * U)

NA = (2, 2, 1, 2)
NF = (2, 2, 2, 2)
HU = len(NA)
NG = H // HU
UPG_A = sum(NA)
UPG_F = sum(NF)
NIF = UPG_F * NG * LT
RVT = max(a + f for a, f in zip(NA, NF))
RV = RVT * 128
V0 = S - RV
A_UNITS = [(hh, RVT - NF[hh] - NA[hh] + j) for hh in range(HU) for j in range(NA[hh])]
F_UNITS = [(hh, RVT - NF[hh] + j) for hh in range(HU) for j in range(NF[hh])]
V_LIST = [(g, j) for g in range(NG) for j in range(UPG_F) if j < UPG_F - 1 or g < 4]
M_LIST = [(g, j) for g in range(NG) for j in range(UPG_F) if (g, j) not in V_LIST]
NIV = len(V_LIST) * LT
IPI = -(-NIV // NB)
RESERVE = 3
CR0 = S - 128 * (NA[HU - 1] + NF[HU - 1]) - 256
KBR = RV // NG
NZ = 2 + UPG_A * LT
TABLE = []
for _n in range(NB * IPI):
    _un, _cb = divmod(min(_n, NIV - 1), LT)
    _g, _j = V_LIST[_un]
    TABLE.append(((_g * UPG_F + _j) * LT + _cb) | ((HU * _g + F_UNITS[_j][0]) << 8) | (F_UNITS[_j][1] << 13))
assert NIF == 256 and H == 32 and LT == 4 and RVT == 4


def _dot(a, b):
    return jnp.dot(a, b, preferred_element_type=F32)


def _dot_nt(a, b):
    return lax.dot_general(a, b, (((1,), (1,)), ((), ())), preferred_element_type=F32)


def _colsum(x, parts):
    if parts > 1:
        x = jnp.sum(x.reshape(x.shape[0] // (8 * parts), 8 * parts, x.shape[1]), axis=0)
    return jnp.sum(x, axis=0, keepdims=True)


def _ln_t(x, parts=1):
    m = _colsum(x, parts) * (1.0 / D)
    xc = x - m
    v = _colsum(xc * xc, parts) * (1.0 / D)
    return xc * lax.rsqrt(v + EPS)


def _rep(col, n):
    return jnp.concatenate([col] * (n // 128), axis=1)


def _kernel(xt_hbm, wmod_hbm, wq_hbm, wo_hbm, c_hbm, wkT_hbm, wvT_hbm, wg_hbm, wu_hbm, wdT_hbm,
            o_ref,
            xt_s, wma_s, wmb_s, wq_s, wo_s,
            modc_s, wqkv_s, woT_s, qt_s, qf_s, k_s, vtf_s, kb_s, pa_s, pf_s, pc_s,
            ot_s, raw_s, ok_s, vok_s, wg_s, wu_s, wdT_s, h2_s, acc_s,
            c_s, cpad_s, wkT_s, wvT_s, zero_s, tab_s, sems, wsems):
    step = pl.program_id(0)

    def w_copies():
        cps = []
        for n in range(NFC):
            for m, (src, dst) in enumerate(((wg_hbm, wg_s), (wu_hbm, wu_s), (wdT_hbm, wdT_s))):
                cps.append(pltpu.make_async_copy(src.at[:, n * FC:(n + 1) * FC], dst.at[n], wsems.at[3 * n + m]))
        return cps

    def x_copy(t):
        return pltpu.make_async_copy(xt_hbm.at[:, t * TQ:(t + 1) * TQ], xt_s.at[t], sems.at[8 + t])

    def mxu_unit(t, kt, h, dst, base):
        r0 = V0 + kt * 128
        s = _dot(k_s[r0:r0 + 128, 0:KP], qt_s[t, h])
        for cb in range(LT):
            dst[base + cb] = jnp.exp2(s[:, cb * 128:(cb + 1) * 128])

    @pl.when(step == 0)
    def _prologue():
        cp_c = pltpu.make_async_copy(c_hbm, c_s, sems.at[0])
        cp_cp = pltpu.make_async_copy(c_hbm.at[:, 0:384], cpad_s, sems.at[1])
        cp_wk = pltpu.make_async_copy(wkT_hbm, wkT_s, sems.at[2])
        cp_wv = pltpu.make_async_copy(wvT_hbm, wvT_s, sems.at[3])
        cp_wq = pltpu.make_async_copy(wq_hbm, wq_s, sems.at[4])
        cp_ma = pltpu.make_async_copy(wmod_hbm.at[:, 0:MA], wma_s, sems.at[5])
        cp_mb = pltpu.make_async_copy(wmod_hbm.at[:, MA:6 * D], wmb_s, sems.at[6])
        cp_wo = pltpu.make_async_copy(wo_hbm, wo_s, sems.at[7])
        for cp in (cp_wq, cp_c, cp_cp, cp_wk, cp_wv, cp_ma):
            cp.start()
        x_copy(0).start()
        for n in range(NZ):
            zero_s[n] = 0
        for n, v in enumerate(TABLE):
            tab_s[n] = v
        pc_s[...] = jnp.zeros_like(pc_s)
        cp_wq.wait()
        wqkv_s[0:D, :] = wq_s[...].astype(F32).T.astype(BF16)
        for cp in (cp_c, cp_cp, cp_wk, cp_wv, cp_ma):
            cp.wait()
        for t in range(1, NQ):
            x_copy(t).start()
        zpad = jnp.zeros((KP - DH, D), F32)
        wqkv_s[D:D + KP, :] = jnp.concatenate([wvT_s[...].astype(F32), zpad], axis=0).astype(BF16)
        wqkv_s[D + KP:D + 2 * KP, :] = jnp.concatenate([wkT_s[...].astype(F32), zpad], axis=0).astype(BF16)
        c = c_s[...].astype(F32)
        sc = c * jax.nn.sigmoid(c)
        sc8 = jnp.broadcast_to(sc, (16, D)).astype(BF16)
        moda = _dot(sc8, wma_s[...])[0:1]
        modc_s[0:MA, :] = jnp.broadcast_to(moda, (128, MA)).T

        qscale = (DH ** -0.5) * LOG2E
        rows = lax.broadcasted_iota(jnp.int32, (KP - 16, TQ), 0)

        def project(t):
            t0 = t * TQ
            sa = _rep(modc_s[0:D, :], TQ)
            ca1 = _rep(modc_s[D:2 * D, :] + 1.0, TQ)
            hT = (_ln_t(xt_s[t].astype(F32), 2) * ca1 + sa).astype(BF16)
            qkv = _dot(wqkv_s[...], hT)
            kT = qkv[D + KP:D + 2 * KP, :]
            kpad = jnp.concatenate([kT, jnp.zeros((128 - KP, TQ), F32)], axis=0)
            k_s[t0:t0 + TQ, :] = kpad.T.astype(BF16)
            for hh in range(H):
                qh = qkv[hh * DH:(hh + 1) * DH, :] * qscale
                qpad = jnp.concatenate([qh, jnp.zeros((KP - DH, TQ), F32)], axis=0).astype(BF16)
                qt_s[t, hh] = qpad
                qpf = qpad.astype(F32)
                for cb in range(LT):
                    qf_s[hh, t * LT + cb, 0:KF, :] = qpf[0:KF, cb * 128:(cb + 1) * 128]
            vt = qkv[D:D + KP, :]
            vhi = jnp.where(rows == DH - 16, 1.0, vt[16:KP, :])
            vb = jnp.concatenate([vt[0:16, :], vhi], axis=0).astype(BF16)
            vtf_s[:, t0:t0 + TQ] = vb.astype(F32)[0:KF]
            vg = jnp.min(jnp.where(jnp.abs(vb.astype(F32)) <= V_HI, 1.0, 0.0).reshape(KP // 8, 8, TQ), axis=0)
            vok_s[...] = vg if t == 0 else jnp.minimum(vok_s[...], vg)

        x_copy(0).wait()
        project(0)
        for t in range(1, NQ):
            x_copy(t).wait()
        cp_mb.start()
        cp_wo.start()
        for t in range(1, NQ):
            project(t)

        def pbody(g, carry):
            for j, (hh, kt) in enumerate(F_UNITS):
                mxu_unit(0, kt, HU * g + hh, pf_s, (UPG_F * g + j) * LT)
            r0 = V0 + g * KBR if isinstance(g, int) else pl.multiple_of(V0 + g * KBR, 16)
            kf = k_s[pl.ds(r0, KBR), :].astype(F32)
            for d in range(DH):
                kb_s[pl.ds(g * (KBR // 16), KBR // 16), :, d] = jnp.broadcast_to(
                    kf[:, d:d + 1], (KBR, 128)).reshape(KBR // 16, 2, 8, 128)
            return carry
        lax.fori_loop(0, NG - 1, pbody, 0)
        cp_mb.wait()
        cp_wo.wait()
        for cp in w_copies():
            cp.start()
        modb = _dot(sc8, wmb_s[...])[0:1]
        modc_s[MA:6 * D, :] = jnp.broadcast_to(modb, (128, 6 * D - MA)).T
        woT_s[...] = wo_s[...].astype(F32).T.astype(BF16)
        pbody(NG - 1, 0)
        for j, (hh, kt) in enumerate(A_UNITS):
            mxu_unit(0, kt, hh, pa_s, j * LT)

    tn = jnp.minimum(step + 1, NQ - 1)
    never = [jnp.full((2, 8, 128), zero_s[n], jnp.int32) != 0 for n in range(2)]

    def vpu_items(items, lag, dc, sg):
        hist = []
        for qfn, kb0, store in items:
            qb = qfn()
            for rb in range(8):
                acc = None
                kbv = kb_s[kb0 + rb]
                for d0 in range(0, DH, dc):
                    prod = kbv[:, d0:d0 + dc] * qb[None, d0:d0 + dc]
                    if acc is None:
                        acc = prod[:, 0]
                        prod = prod[:, 1:]
                        if lag and len(hist) >= lag:
                            acc = jnp.where(never[1], hist[-lag][1], acc)
                        if hist:
                            acc = jnp.where(never[0], hist[-1][0], acc)
                    acc = jnp.sum(jnp.concatenate([acc[:, None], prod], axis=1), axis=1)
                hist.append((acc, jnp.exp2(acc)))
                if (rb + 1) % sg == 0:
                    store((rb + 1 - sg) * 16, jnp.concatenate([h[1] for h in hist[-sg:]], axis=0).reshape(16 * sg, 128))

    def bcast_q(h, lt):
        q = qf_s[h, lt, 0:KF, :]
        return jnp.stack([jnp.broadcast_to(q[d:d + 1, :], (8, 128)) for d in range(DH)], axis=0)

    def norm(oT):
        l = oT[DH:DH + 1, :]
        return oT[0:DH, :] * (1.0 / l), l

    ok_s[...] = vok_s[...]
    raw_s[...] = jnp.ones_like(raw_s)

    def finish(i, live):
        extra = _dot(vtf_s[:, CR0:CR0 + 256], pc_s[...])
        outs = []
        ok = ok_s[...]
        for hh in range(HU):
            raw = raw_s[hh]
            if hh == HU - 1:
                raw = raw + jnp.where(live, extra, 0.0)
            o, l = norm(raw)
            outs.append(o)
            ok = jnp.where(jnp.logical_and(l >= L_LO, l <= L_HI), ok, 0.0)
        ok_s[...] = ok
        r0 = pl.multiple_of(i * (HU * DH), 8)
        ot_s[pl.ds(r0, HU * DH), :] = jnp.concatenate(outs, axis=0)

    def abody(i, carry):
        qTs = [qt_s[step, HU * i + hh] for hh in range(HU)]
        oT = [None] * HU

        def add(hh, v):
            oT[hh] = v if oT[hh] is None else oT[hh] + v

        def unit_tile(kind, j):
            hh, kt = (A_UNITS if kind == "a" else F_UNITS)[j]

            def get():
                if kind == "a":
                    return jnp.concatenate([pa_s[j * LT + cb] for cb in range(LT)], axis=1)
                return jnp.concatenate([pf_s[(UPG_F * i + j) * LT + cb] for cb in range(LT)], axis=1)
            return (hh, V0 + kt * 128, get)

        def pv(tiles):
            if len(tiles) == 2 and tiles[0][0] == tiles[1][0]:
                v = jnp.concatenate([vtf_s[:, t[1]:t[1] + 128] for t in tiles], axis=1)
                add(tiles[0][0], _dot(v, jnp.concatenate([t[2]() for t in tiles], axis=0)))
            else:
                for hh, r0, get in tiles:
                    add(hh, _dot(vtf_s[:, r0:r0 + 128], get()))

        units = [unit_tile("a", j) for j in range(UPG_A)] + [unit_tile("f", j) for j in reversed(range(UPG_F))]
        tail = units[len(units) - RESERVE:]
        units = units[:len(units) - RESERVE]
        ready = []

        def unit_pair():
            for n, u in enumerate(units):
                for m in range(n + 1, len(units)):
                    if units[m][0] == u[0]:
                        b = units.pop(m)
                        return [units.pop(n), b]
            return None

        for hh in range(HU):
            rows = 256 - 16 * (NA[hh] + NF[hh])
            buf = None
            r0 = 0
            for k in range(8):
                p = jnp.exp2(_dot(k_s[k * rows:(k + 1) * rows, 0:KP], qTs[hh]))
                if len(ready) >= 2:
                    pv([ready.pop(0), ready.pop(0)])
                elif ready:
                    pv([ready.pop(0)] + ([units.pop(0)] if units else []))
                else:
                    assert hh == 0 and k == 0
                    finish(jnp.maximum(i - 1, 0), i > 0)
                buf = p if buf is None else jnp.concatenate([buf, p], axis=0)
                while buf is not None and buf.shape[0] >= 128:
                    ready.append((hh, r0, lambda v=buf[0:128]: v))
                    r0 += 128
                    buf = buf[128:] if buf.shape[0] > 128 else None
            assert buf is None
        units.extend(tail)
        while units:
            up = unit_pair()
            pv(up if up is not None else [units.pop(0)])
        assert len(ready) == 2 and ready[0][1] == CR0
        pc_s[...] = jnp.concatenate([ready[0][2](), ready[1][2]()], axis=0)

        last = i == NG - 1
        gn = jnp.where(last, 0, i + 1)
        tsn = jnp.where(last, tn, step)
        cache = {}
        items = []
        for j, (hh, kt) in enumerate(A_UNITS):
            for cb in range(LT):
                def qfn(hh=hh, cb=cb):
                    if (hh, cb) not in cache:
                        cache[(hh, cb)] = bcast_q(HU * gn + hh, tsn * LT + cb)
                    return cache[(hh, cb)]

                def store(rr, val, j=j, cb=cb):
                    pa_s[j * LT + cb, rr:rr + val.shape[0], :] = val
                kb0 = ((kt + zero_s[2 + j * LT + cb]) & (RVT - 1)) * 8
                items.append(((hh, cb, j), (qfn, kb0, store)))
        items.sort(key=lambda x: x[0])
        vpu_items([it for _, it in items], 2, 2, 8)
        for hh in range(HU):
            raw_s[hh] = oT[hh]
        return carry
    lax.fori_loop(0, NG, abody, 0)

    def safe_attn():
        def body(i, carry):
            def hbody(hh, c2):
                sT = _dot(k_s[:, 0:KP], qt_s[step, HU * i + hh])
                m = jnp.max(sT, axis=0, keepdims=True)
                raw_s[hh] = _dot(vtf_s[...], jnp.exp2(sT - m))
                return c2
            lax.fori_loop(0, HU, hbody, 0)
            r0 = pl.multiple_of(i * (HU * DH), 8)
            ot_s[pl.ds(r0, HU * DH), :] = jnp.concatenate([norm(raw_s[hh])[0] for hh in range(HU)], axis=0)
            return carry
        lax.fori_loop(0, NG, body, 0)

    def mid():
        attnT = _dot(woT_s[...], ot_s[...].astype(BF16))
        ga = _rep(modc_s[2 * D:3 * D, :], TQ)
        sb = _rep(modc_s[3 * D:4 * D, :], TQ)
        cb1 = _rep(modc_s[4 * D:5 * D, :] + 1.0, TQ)
        x1 = xt_s[step].astype(F32) + ga * attnT
        acc_s[...] = x1
        h2T = _ln_t(x1) * cb1 + sb
        h2_s[...] = h2T.T.astype(BF16)
        for g, j in M_LIST:
            hh, kt = F_UNITS[j]
            mxu_unit(tn, kt, HU * g + hh, pf_s, (UPG_F * g + j) * LT)

    def mbody(c):
        pl.when(c == 1)(safe_attn)
        finish(NG - 1, c == 0)
        bad = jnp.min(ok_s[...]) < 0.5
        mid()
        return jnp.where(jnp.logical_and(c == 0, bad), 1, 2)
    lax.while_loop(lambda c: c < 2, mbody, jnp.int32(0))

    @pl.when(step == 0)
    def _():
        for cp in w_copies():
            cp.wait()

    def fbody(b, carry):
        h2 = h2_s[...]

        def gu(j):
            return _dot(h2, wg_s[b * U + j]), _dot(h2, wu_s[b * U + j])
        acc = None
        nxt = gu(0)
        for j in range(U):
            g, u = nxt
            if j + 1 < U:
                nxt = gu(j + 1)
            hg = 0.5 * g
            act = ((hg * u) * (1.0 + jnp.tanh(hg))).astype(BF16)
            dn = _dot_nt(wdT_s[b * U + j], act)
            acc = dn if acc is None else acc + dn
        gb = _rep(modc_s[5 * D:6 * D, :], TQ)
        acc_s[...] += gb * acc
        items = []
        for jj in range(IPI):
            e = tab_s[b * IPI + jj]

            def qfn(h=(e >> 8) & (H - 1), lt=tn * LT + (e & (LT - 1))):
                return bcast_q(h, lt)

            def store(rr, val, it=e & (NIF - 1)):
                pf_s[it, rr:rr + val.shape[0], :] = val
            items.append((qfn, ((e >> 13) & (RVT - 1)) * 8, store))
        vpu_items(items, 0, 6, 4)
        return carry
    lax.fori_loop(0, NB, fbody, 0)
    o_ref[...] = acc_s[...].astype(o_ref.dtype)


@jax.jit
def pallas_adaLN_cond__grouped_kv_mqa__swiglu_ffn__prompt_kernel(
    A_x: jax.Array,
    A_wq: jax.Array,
    A_wk: jax.Array,
    A_wv: jax.Array,
    A_wo: jax.Array,
    B_x: jax.Array,
    B_w_gate: jax.Array,
    B_w_up: jax.Array,
    B_w_down: jax.Array,
    c: jax.Array,
    w_mod: jax.Array,
):
    del B_x
    xT = A_x.reshape(S, D).T
    hbm = pl.BlockSpec(memory_space=pl.ANY)
    outT = pl.pallas_call(
        _kernel,
        grid=(NQ,),
        in_specs=[hbm] * 10,
        out_specs=pl.BlockSpec((D, TQ), lambda i: (0, i)),
        out_shape=jax.ShapeDtypeStruct((D, S), BF16),
        scratch_shapes=[
            pltpu.VMEM((NQ, D, TQ), BF16),
            pltpu.VMEM((D, MA), BF16),
            pltpu.VMEM((D, 6 * D - MA), BF16),
            pltpu.VMEM((D, D), BF16),
            pltpu.VMEM((D, D), BF16),
            pltpu.VMEM((6 * D, 128), F32),
            pltpu.VMEM((D + 2 * KP, D), BF16),
            pltpu.VMEM((D, D), BF16),
            pltpu.VMEM((NQ, H, KP, TQ), BF16),
            pltpu.VMEM((H, S // 128, KP, 128), F32),
            pltpu.VMEM((S, 128), BF16),
            pltpu.VMEM((KF, S), F32),
            pltpu.VMEM((RV // 16, 2, DH, 8, 128), F32),
            pltpu.VMEM((UPG_A * LT, 128, 128), F32),
            pltpu.VMEM((NIF, 128, 128), F32),
            pltpu.VMEM((256, TQ), F32),
            pltpu.VMEM((D, TQ), F32),
            pltpu.VMEM((HU, KF, TQ), F32),
            pltpu.VMEM((8, TQ), F32),
            pltpu.VMEM((8, TQ), F32),
            pltpu.VMEM((NFC, D, FC), BF16),
            pltpu.VMEM((NFC, D, FC), BF16),
            pltpu.VMEM((NFC, D, FC), BF16),
            pltpu.VMEM((TQ, D), BF16),
            pltpu.VMEM((D, TQ), F32),
            pltpu.VMEM((1, D), BF16),
            pltpu.VMEM((1, 384), BF16),
            pltpu.VMEM((DH, D), BF16),
            pltpu.VMEM((DH, D), BF16),
            pltpu.SMEM((NZ,), jnp.int32),
            pltpu.SMEM((len(TABLE),), jnp.int32),
            pltpu.SemaphoreType.DMA((8 + NQ,)),
            pltpu.SemaphoreType.DMA((3 * NFC,)),
        ],
        compiler_params=pltpu.CompilerParams(
            dimension_semantics=("arbitrary",),
            vmem_limit_bytes=110 * 1024 * 1024),
    )(xT, w_mod, A_wq, A_wo, c, A_wk.T, A_wv.T, B_w_gate, B_w_up, B_w_down.T)
    return outT.T.reshape(1, S, D)
```
